```python
import os as _os
_os.environ.setdefault("JAX_PLATFORMS", "cpu")
import jax
import jax.numpy as jnp

def _softmax(x, axis=-1):
    return jax.nn.softmax(x, axis=axis)
def _gelu(x):
    return jax.nn.gelu(x, approximate=True)
def _silu(x):
    return jax.nn.silu(x)
def _sigmoid(x):
    return jax.nn.sigmoid(x)
def _layernorm(x, axis=-1, eps=1e-5):
    m = jnp.mean(x, axis=axis, keepdims=True)
    v = jnp.var(x, axis=axis, keepdims=True)
    return (x - m) / jnp.sqrt(v + eps)
def _scatter_add(tgt, idx, src, axis=0):
    return tgt.at[idx].add(src)
def _segment_sum(src, seg, n):
    return jax.ops.segment_sum(src, seg, n)
class _Rng:
    def __init__(self, key):
        self._k = key
    def _next(self):
        self._k, sub = jax.random.split(self._k)
        return sub
    def normal(self, shape):
        return jax.random.normal(self._next(), shape, dtype=jnp.bfloat16)
    def randint(self, lo, hi, shape):
        return jax.random.randint(self._next(), shape, lo, hi, dtype=jnp.int32)
    def uniform(self, shape, lo=0.0, hi=1.0):
        return jax.random.uniform(self._next(), shape, jnp.bfloat16, lo, hi)
    def permutation(self, n):
        return jax.random.permutation(self._next(), n)


kernel_name = 'gated_mix__linear_attn_block__mixer_token_mlp__prompt'

def setup_inputs():
    _rng = _Rng(jax.random.key(int.from_bytes(__import__("os").urandom(4), "little")))
    _w = (lambda a: (lambda t: t.astype(jnp.bfloat16) if jnp.issubdtype(t.dtype, jnp.floating) else t)(jnp.asarray(a)))
    def _A_setup():
        B, S, D = 1, 2048, 512
        return {
            "x": _w((lambda *s: _rng.normal(s) * 0.05)(B, S, D)),
            "wqkv": _w((lambda *s: _rng.normal(s) * 0.8)(D, 3 * D)),
            "wo": _w((lambda *s: _rng.normal(s) * 0.05)(D, D)),
        }
    _A_in = _A_setup()

    def _B_setup():
        B, S, D, F = 1, 2048, 512, 1792
        return {
            "x": _w((lambda *s: _rng.normal(s) * 0.05)(B, S, D)),
            "w1": _w((lambda *s: _rng.normal(s) * 0.1)(S, F) * (S ** -0.5)),
            "b1": _w((lambda *s: _rng.normal(s) * 0.1)(F) * 0.02),
            "w2": _w((lambda *s: _rng.normal(s) * 0.1)(F, S) * (F ** -0.5)),
            "b2": _w((lambda *s: _rng.normal(s) * 0.1)(S) * 0.02),
        }
    _B_in = _B_setup()

    return {
        "A_x": _A_in["x"],
        "A_wqkv": _A_in["wqkv"],
        "A_wo": _A_in["wo"],
        "B_x": _B_in["x"],
        "B_w1": _B_in["w1"],
        "B_b1": _B_in["b1"],
        "B_w2": _B_in["w2"],
        "B_b2": _B_in["b2"],
        "gate_w": _w((lambda *s: _rng.normal(s) * 0.05)(512) * 16.0),
    }

def reference(A_x, A_wqkv, A_wo, B_x, B_w1, B_b1, B_w2, B_b2, gate_w):
    def _A_ref(x, wqkv, wo):
        B, S, D = x.shape
        H = 32; Dh = D // H
        qkv = (lambda x, *d: x.transpose(*d))((x @ wqkv).reshape(B, S, 3, H, Dh), 2, 0, 3, 1, 4)
        q, k, v = qkv[0], qkv[1], qkv[2]
        phi = lambda t: jnp.where(t > 0, t + 1, jnp.exp(t)) + 1e-6
        pq, pk = phi(q), phi(k)
        kv = jnp.einsum("bhsd,bhse->bhde", pk, v)
        z = jnp.einsum("bhsd->bhd", pk)
        num = jnp.einsum("bhqd,bhde->bhqe", pq, kv)
        den = jnp.einsum("bhqd,bhd->bhq", pq, z)[..., None] + 1e-6
        o = num / den
        return (lambda x, *d: x.transpose(*d))(o, 0, 2, 1, 3).reshape(B, S, D) @ wo

    def _B_ref(x, w1, b1, w2, b2):
        B, S, D = x.shape
        h = _layernorm(x, axis=-1)
        u = jnp.einsum("bsd,sf->bdf", h, w1) + b1
        u = _gelu(u)
        y = jnp.einsum("bdf,fs->bds", u, w2) + b2
        return (lambda x, *d: x.transpose(*d))(y, 0, 2, 1)

    x = A_x
    g = _sigmoid((x * gate_w).sum(-1, keepdims=True))
    a = _A_ref(x, A_wqkv, A_wo)
    b = _B_ref(x, B_w1, B_b1, B_w2, B_b2)
    return g * a + (1 - g) * b
```

```python
import functools
import jax
import jax.numpy as jnp
from jax import lax
import jax.experimental.pallas as pl
import jax.experimental.pallas.tpu as pltpu

S, D, F, H, DH = 2048, 512, 1792, 32, 16
f32, bf16 = jnp.float32, jnp.bfloat16
NT = (((1,), (1,)), ((), ()))
NN = (((1,), (0,)), ((), ()))

def dot(a, b, dn=NN):
    return lax.dot_general(a, b, dn, preferred_element_type=f32)

def phi(t):
    return jnp.where(t > 0, t + 1.0, jnp.exp(t)) + 1e-6

def gelu(x):
    c = 0.7978845608028654
    return 0.5 * x * (1.0 + jnp.tanh(c * (x + 0.044715 * (x * x * x))))

TC = 512
FC = 256
OC = 256

def kernel(ax_h, wqkv_h, wo_h, bx_h, w1_h, b1_h, w2_h, b2_h, gw_h, out_h,
           ax_v, wqkv_v, wo_v, bx_v, w1_v, w2_v, b1_v, b2_v, gw_v,
           wqg, wkT, woT, hT, pqT, pkT, G, zc, gT, gu, mT, out_v, b12, sems, osems):
    ncp1 = S // TC
    sem_i = [0]
    def cp(src, dst):
        i = sem_i[0]; sem_i[0] += 1
        return pltpu.make_async_copy(src, dst, sems.at[i])
    c_wqk = cp(wqkv_h.at[:, pl.ds(0, 2 * D)], wqkv_v.at[:, pl.ds(0, 2 * D)])
    c_gw = cp(gw_h, gw_v)
    c_ax = [cp(ax_h.at[pl.ds(c * TC, TC)], ax_v.at[pl.ds(c * TC, TC)]) for c in range(ncp1)]
    c_wv = cp(wqkv_h.at[:, pl.ds(2 * D, D)], wqkv_v.at[:, pl.ds(2 * D, D)])
    c_wo = cp(wo_h, wo_v)
    c_b1 = cp(b1_h, b1_v)
    c_b2 = cp(b2_h, b2_v)
    c_w1 = [cp(w1_h.at[:, pl.ds(j * FC, FC)], w1_v.at[:, pl.ds(j * FC, FC)]) for j in range(F // FC)]
    c_w2 = [cp(w2_h.at[:, pl.ds(j * OC, OC)], w2_v.at[:, pl.ds(j * OC, OC)]) for j in range(S // OC)]
    c_wqk.start(); c_gw.start()
    for c in range(ncp1):
        c_ax[c].start()
    c_wv.start(); c_wo.start(); c_b1.start(); c_b2.start()
    for c in c_w1: c.start()
    for c in c_w2: c.start()

    c_wqk.wait(); c_gw.wait()
    wqg[pl.ds(0, D), :] = wqkv_v[:, pl.ds(0, D)].T
    wkT[...] = wqkv_v[:, pl.ds(D, D)].T
    gwrow = gw_v[...].astype(f32).reshape(1, D)
    rid = lax.broadcasted_iota(jnp.int32, (16, D), 0)
    wqg[pl.ds(D, 16), :] = jnp.where(rid == 0, jnp.broadcast_to(gwrow, (16, D)), 0.0).astype(bf16)

    G[...] = jnp.zeros_like(G)
    zc[...] = jnp.zeros_like(zc)

    for c in range(ncp1):
        c_ax[c].wait()
        cs = pl.ds(c * TC, TC)
        x_c = ax_v[cs, :]
        xT = x_c.T
        qg = dot(wqg[...], xT)
        pqT[:, cs] = phi(qg[:D]).astype(bf16)
        gT[:, cs] = jax.nn.sigmoid(qg[D:D + 8])
        k = dot(wkT[...], xT)
        pk = phi(k)
        zc[...] += pk[:, 0:128] + pk[:, 128:256] + pk[:, 256:384] + pk[:, 384:512]
        pkb = pk.astype(bf16)
        G[...] += dot(pkb, x_c)
        xb = xT.astype(f32)
        m = jnp.mean(xb, axis=0, keepdims=True)
        xc = xb - m
        v = jnp.mean(xc * xc, axis=0, keepdims=True)
        hT[:, cs] = (xc * lax.rsqrt(v + 1e-5)).astype(bf16)

    c_wv.wait(); c_wo.wait(); c_b1.wait(); c_b2.wait()
    b12[0:1, pl.ds(0, F)] = b1_v[...].astype(f32).reshape(1, F)
    b12[1:2, :] = b2_v[...].astype(f32).reshape(1, S)
    woT[...] = wo_v[...].T
    zcol = jnp.sum(zc[...], axis=1, keepdims=True)
    zc[...] = jnp.broadcast_to(zcol, (D, 128))
    r = lax.broadcasted_iota(jnp.int32, (128, 128), 0) // DH
    cc = lax.broadcasted_iota(jnp.int32, (128, 128), 1) // DH
    for g in range(4):
        gs = pl.ds(g * 128, 128)
        kv = dot(G[gs, :].astype(bf16), wqkv_v[:, pl.ds(2 * D + g * 128, 128)])
        kvb = jnp.where(r == cc, kv, 0.0).astype(bf16)
        mT[:, gs] = dot(woT[:, gs], kvb, NT).astype(bf16)

    def p3(j, carry):
        js = pl.ds(pl.multiple_of(j * FC, FC), FC)
        u = dot(hT[...], w1_v[:, js]) + b12[0:1, js]
        gu[:, js] = gelu(u).astype(bf16)
        return carry
    for j in range(F // FC):
        c_w1[j].wait()
        p3(j, 0)

    for j in range(S // OC):
        c_w2[j].wait()
        js = pl.ds(j * OC, OC)
        pq = pqT[:, js].astype(f32)
        pz = pq * jnp.tile(zc[...], (1, OC // 128))
        den = jnp.sum(pz.reshape(H, DH, OC), axis=1, keepdims=True) + 1e-6
        g = gT[0:1, js]
        sc = (g.reshape(1, 1, OC) / den)
        pqn = (pq.reshape(H, DH, OC) * sc).reshape(D, OC).astype(bf16)
        a = dot(mT[...], pqn)
        y = dot(gu[...], w2_v[:, js]) + b12[1:2, js]
        o = (a + (1.0 - g) * y).astype(bf16)
        slot = j % 2
        if j >= 2:
            pltpu.make_async_copy(out_v.at[slot], out_h.at[pl.ds((j - 2) * OC, OC)], osems.at[slot]).wait()
        out_v[slot] = o.T
        pltpu.make_async_copy(out_v.at[slot], out_h.at[pl.ds(j * OC, OC)], osems.at[slot]).start()
    n5 = S // OC
    for j in (n5 - 2, n5 - 1):
        pltpu.make_async_copy(out_v.at[j % 2], out_h.at[pl.ds(j * OC, OC)], osems.at[j % 2]).wait()


@jax.jit
def pallas_gated_mix__linear_attn_block__mixer_token_mlp__prompt_kernel(
        A_x, A_wqkv, A_wo, B_x, B_w1, B_b1, B_w2, B_b2, gate_w):
    any_spec = pl.BlockSpec(memory_space=pl.ANY)
    V = pltpu.VMEM
    scratch = [
        V((S, D), bf16), V((D, 3 * D), bf16), V((D, D), bf16), V((S, D), bf16),
        V((S, F), bf16), V((F, S), bf16), V((F,), bf16), V((S,), bf16), V((D,), bf16),
        V((D + 16, D), bf16), V((D, D), bf16), V((D, D), bf16),
        V((D, S), bf16), V((D, S), bf16), V((D, S), bf16),
        V((D, D), f32), V((D, 128), f32), V((8, S), f32),
        V((D, F), bf16), V((D, D), bf16), V((2, OC, D), bf16), V((8, S), f32),
        pltpu.SemaphoreType.DMA((40,)), pltpu.SemaphoreType.DMA((2,)),
    ]
    out = pl.pallas_call(
        kernel,
        in_specs=[any_spec] * 9,
        out_specs=any_spec,
        out_shape=jax.ShapeDtypeStruct((S, D), bf16),
        scratch_shapes=scratch,
        compiler_params=pltpu.CompilerParams(vmem_limit_bytes=100 * 1024 * 1024),
    )(A_x.reshape(S, D), A_wqkv, A_wo, B_x.reshape(S, D), B_w1, B_b1, B_w2, B_b2, gate_w)
    return out.reshape(1, S, D)
```

```python
import functools
import jax
import jax.numpy as jnp
from jax import lax
import jax.experimental.pallas as pl
import jax.experimental.pallas.tpu as pltpu

S, D, F, H, DH = 2048, 512, 1792, 32, 16
f32, bf16 = jnp.float32, jnp.bfloat16
NT = (((1,), (1,)), ((), ()))
NN = (((1,), (0,)), ((), ()))

def dot(a, b, dn=NN):
    return lax.dot_general(a, b, dn, preferred_element_type=f32)

def phi(t):
    return jnp.where(t > 0, t + 1.0, jnp.exp(t)) + 1e-6

def gelu(x):
    c = 0.7978845608028654
    return 0.5 * x * (1.0 + jnp.tanh(c * (x + 0.044715 * (x * x * x))))

TC = 512
FC = 256
OC = 256
NC = S // TC
SEQ = "GW T:0 K:0 G:0|K:1 WQ T:1 Q:0 Q:1 G:1|T:2 K:2 Q:2 G:2 T:3 K:3 Q:3 G:3 WV WO B12".split("|")

def kernel(x_h, wqkv_h, wo_h, w1_h, b1_h, w2_h, b2_h, gw_h, out_h,
           x_v, wqkv_v, wo_v, w1_v, w2_v, b1_v, b2_v, gw_v,
           wqT, wvT, woT, xT, hT, pqT, pk, Gt, zr, zc, gwc, gT, gu, mT, out_v, b12, st, sems, osems):
    sem_i = [0]
    def cp(src, dst):
        i = sem_i[0]; sem_i[0] += 1
        return pltpu.make_async_copy(src, dst, sems.at[i])
    c_wk = cp(wqkv_h.at[:, pl.ds(D, D)], wqkv_v.at[:, pl.ds(D, D)])
    c_x = [cp(x_h.at[pl.ds(c * TC, TC)], x_v.at[pl.ds(c * TC, TC)]) for c in range(NC)]
    c_wq = cp(wqkv_h.at[:, pl.ds(0, D)], wqkv_v.at[:, pl.ds(0, D)])
    c_gw = cp(gw_h, gw_v)
    c_wv = cp(wqkv_h.at[:, pl.ds(2 * D, D)], wqkv_v.at[:, pl.ds(2 * D, D)])
    c_wo = cp(wo_h, wo_v)
    c_b1 = cp(b1_h, b1_v)
    c_b2 = cp(b2_h, b2_v)
    c_w1 = [cp(w1_h.at[pl.ds(c * TC, TC)], w1_v.at[pl.ds(c * TC, TC)]) for c in range(NC)]
    c_w2 = [cp(w2_h.at[:, pl.ds(j * (S // 2), S // 2)], w2_v.at[:, pl.ds(j * (S // 2), S // 2)]) for j in range(2)]
    for c in [c_wk, c_x[0], c_gw, c_wq, c_x[1], c_x[2], c_x[3], c_wv, c_wo, c_b1, c_b2] + c_w1 + c_w2:
        c.start()

    def K(c):
        cs = pl.ds(c * TC, TC)
        k = dot(x_v[cs, :], wqkv_v[:, pl.ds(D, D)])
        p = phi(k)
        zpart = jnp.sum(p.reshape(TC // 8, 8, D), axis=0)
        if c == 0:
            zr[...] = zpart
        else:
            zr[...] += zpart
        pk[cs, :] = p.astype(bf16)

    def T(c):
        cs = pl.ds(c * TC, TC)
        xT[:, cs] = x_v[cs, :].T

    def LN(c, n=1):
        pass

    def WQ():
        wqT[pl.ds(0, D), :] = wqkv_v[:, pl.ds(0, D)].T
    def GW():
        gwrow = jnp.broadcast_to(gw_v[...].astype(f32).reshape(1, D), (16, D))
        rid = lax.broadcasted_iota(jnp.int32, (16, D), 0)
        wqT[pl.ds(D, 16), :] = jnp.where(rid == 0, 1.0 / D, jnp.where(rid == 1, gwrow, 0.0)).astype(bf16)
    def WV():
        wvT[...] = wqkv_v[:, pl.ds(2 * D, D)].T
    def WO():
        woT[...] = wo_v[...].T
    def B12():
        b12[0:1, pl.ds(0, F)] = b1_v[...].astype(f32).reshape(1, F)
        b12[1:2, :] = b2_v[...].astype(f32).reshape(1, S)
    ops = dict(K=K, T=T, LN=LN, WQ=WQ, GW=GW, WV=WV, WO=WO, B12=B12)
    def run(seq):
        for item in seq.split():
            name, _, arg = item.partition(":")
            args = [int(a) for a in arg.split(",")] if arg else []
            ops[name](*args)

    def GATE(c):
        cs = pl.ds(c * TC, TC)
        xb = xT[:, cs].astype(f32)
        gl = jnp.sum(xb * jnp.tile(gwc[...], (1, TC // 128)), axis=0, keepdims=True)
        gT[0:1, cs] = jax.nn.sigmoid(gl)

    def Q(c):
        cs = pl.ds(c * TC, TC)
        q = dot(wqT[...], xT[:, cs])
        pqT[:, cs] = phi(q[:D]).astype(bf16)
        mg = q[D:D + 8]
        gT[:, cs] = jax.nn.sigmoid(mg)
        for l in range(TC // 128):
            ls = pl.ds(c * TC + l * 128, 128)
            m = mg[0:1, l * 128:(l + 1) * 128]
            xc = xT[:, ls].astype(f32) - m
            v = jnp.sum(xc * xc, axis=0, keepdims=True) * (1.0 / D)
            r = lax.rsqrt(v + 1e-5)
            hT[:, ls] = ((xT[:, ls].astype(f32) - m) * r).astype(bf16)

    def G(c, n=1):
        cs = pl.ds(c * TC, n * TC)
        r = dot(xT[:, cs], pk[cs, :])
        if c == 0:
            Gt[...] = r
        else:
            Gt[...] += r

    ops.update(Q=Q, G=G)
    c_wk.wait(); c_x[0].wait(); c_gw.wait()
    run(SEQ[0])
    c_wq.wait(); c_x[1].wait()
    run(SEQ[1])
    c_x[2].wait(); c_x[3].wait(); c_wv.wait(); c_wo.wait(); c_b1.wait(); c_b2.wait()
    run(SEQ[2])
    for c in c_w1: c.wait()
    zrow = jnp.sum(zr[...], axis=0, keepdims=True)
    zc[...] = jnp.broadcast_to(zrow, (128, D)).T
    r = lax.broadcasted_iota(jnp.int32, (128, 128), 0) // DH
    cc = lax.broadcasted_iota(jnp.int32, (128, 128), 1) // DH
    for g in range(4):
        gs = pl.ds(g * 128, 128)
        kvT = dot(wvT[gs, :], Gt[:, gs].astype(bf16))
        kvb = jnp.where(r == cc, kvT, 0.0).astype(bf16)
        mT[:, gs] = dot(woT[:, gs], kvb).astype(bf16)
    for j in range(F // FC):
        js = pl.ds(j * FC, FC)
        u = dot(hT[...], w1_v[:, js]) + b12[0:1, js]
        gu[:, js] = gelu(u).astype(bf16)

    def P5(j):
        js = pl.ds(j * OC, OC)
        y = dot(gu[...], w2_v[:, js]) + b12[1:2, js]
        pq = pqT[:, js].astype(f32)
        pz = pq * jnp.tile(zc[...], (1, OC // 128))
        den = jnp.sum(pz.reshape(H, DH, OC), axis=1, keepdims=True) + 1e-6
        g = gT[1:2, js]
        sc = (g.reshape(1, 1, OC) / den)
        pqn = (pq.reshape(H, DH, OC) * sc).reshape(D, OC).astype(bf16)
        a = dot(mT[...], pqn)
        o = (a + (1.0 - g) * y).astype(bf16)
        out_v[js, :] = o.T
    def ocp(i, lo, n):
        js = pl.ds(lo, n)
        return pltpu.make_async_copy(out_v.at[js], out_h.at[js], osems.at[i])
    n5 = S // OC
    c_w2[0].wait()
    for j in range(n5 // 2): P5(j)
    ocp(0, 0, S // 2).start()
    c_w2[1].wait()
    for j in range(n5 // 2, n5 - 1): P5(j)
    ocp(1, S // 2, S // 2 - OC).start()
    ocp(0, 0, S // 2).wait()
    P5(n5 - 1)
    ocp(2, S - OC, OC).start()
    ocp(1, S // 2, S // 2 - OC).wait()
    ocp(2, S - OC, OC).wait()


@jax.jit
def pallas_gated_mix__linear_attn_block__mixer_token_mlp__prompt_kernel(
        A_x, A_wqkv, A_wo, B_x, B_w1, B_b1, B_w2, B_b2, gate_w):
    any_spec = pl.BlockSpec(memory_space=pl.ANY)
    V = pltpu.VMEM
    scratch = [
        V((S, D), bf16), V((D, 3 * D), bf16), V((D, D), bf16),
        V((S, F), bf16), V((F, S), bf16), V((F,), bf16), V((S,), bf16), V((D,), bf16),
        V((D + 16, D), bf16), V((D, D), bf16), V((D, D), bf16),
        V((D, S), bf16), V((D, S), bf16), V((D, S), bf16), V((S, D), bf16),
        V((D, D), f32), V((8, D), f32), V((D, 128), f32), V((D, 128), f32), V((8, S), f32),
        V((D, F), bf16), V((D, D), bf16), V((S, D), bf16), V((8, S), f32), V((8, S), f32),
        pltpu.SemaphoreType.DMA((24,)), pltpu.SemaphoreType.DMA((4,)),
    ]
    out = pl.pallas_call(
        kernel,
        in_specs=[any_spec] * 8,
        out_specs=any_spec,
        out_shape=jax.ShapeDtypeStruct((S, D), bf16),
        scratch_shapes=scratch,
        compiler_params=pltpu.CompilerParams(vmem_limit_bytes=100 * 1024 * 1024),
    )(A_x.reshape(S, D), A_wqkv, A_wo, B_w1, B_b1, B_w2, B_b2, gate_w)
    return out.reshape(1, S, D)
```

```python
import jax
import jax.numpy as jnp
from jax import lax
import jax.experimental.pallas as pl
import jax.experimental.pallas.tpu as pltpu

S, D, F, H, DH = 2048, 512, 1792, 32, 16
FC = 256
f32, bf16, i32 = jnp.float32, jnp.bfloat16, jnp.int32


def _dot(a, b):
    return lax.dot_general(a, b, (((1,), (0,)), ((), ())), preferred_element_type=f32)


def _phi(t):
    return jnp.where(t > 0, t + 1.0, jnp.exp(t)) + 1e-6


def _gelu(x):
    c = 0.7978845608028654
    return 0.5 * x * (1.0 + jnp.tanh(c * (x + 0.044715 * (x * x * x))))


def _pack(v):
    return pltpu.bitcast(v, i32)


def _unpack(v):
    return pltpu.bitcast(v, bf16)


def _after(v):
    return jnp.minimum(jnp.abs(v), 1.0) * 0.0


def _kernel(x_h, wqkv_h, wo_h, w1_h, b1_h, w2_h, b2_h, gw_h,
            out_h,
            x_v, wqkv_v, wo_v, w1_v, w2_v, b1_v, b2_v, gw_v,
            wqT, wvT, woT, xT, hT, pqT, pk,
            Gt, zr, zc, gwc, gT, b12, aT,
            kvb, mT, gu, out_v,
            in_sems, out_sems):

    cps = {}

    def fetch(name, src, dst):
        cps[name] = pltpu.make_async_copy(src, dst, in_sems.at[len(cps)])
        cps[name].start()

    def wait(*names):
        for n in names:
            cps[n].wait()

    def rows(name, h, v, lo, n):
        fetch(name, h.at[pl.ds(lo, n)], v.at[pl.ds(lo, n)])

    def cols(name, h, v, lo, n):
        fetch(name, h.at[:, pl.ds(lo, n)], v.at[:, pl.ds(lo, n)])

    cols("wk0", wqkv_h, wqkv_v, D, 256)
    rows("x0", x_h, x_v, 0, 256)
    cols("wk1", wqkv_h, wqkv_v, D + 256, 256)
    rows("x1", x_h, x_v, 256, 256)
    fetch("gw", gw_h, gw_v)
    cols("wq", wqkv_h, wqkv_v, 0, D)
    rows("x2", x_h, x_v, 512, 512)
    rows("x3", x_h, x_v, 1024, 512)
    rows("x4", x_h, x_v, 1536, 512)
    cols("wv", wqkv_h, wqkv_v, 2 * D, D)
    fetch("wo", wo_h, wo_v)
    fetch("b1", b1_h, b1_v)
    fetch("b2", b2_h, b2_v)
    fetch("w1", w1_h, w1_v)
    cols("w2a", w2_h, w2_v, 0, S // 2)
    cols("w2b", w2_h, w2_v, S // 2, S // 2)

    seen_z, seen_g = set(), set()

    def K(t0, nt, n0, nn):
        k = _dot(x_v[pl.ds(t0, nt), :], wqkv_v[:, pl.ds(D + n0, nn)])
        p = _phi(k)
        zpart = jnp.sum(p.reshape(nt // 8, 8, nn), axis=0)
        for n in range(n0, n0 + nn, 128):
            zp = zpart[:, n - n0:n - n0 + 128]
            if n not in seen_z:
                seen_z.add(n)
                zr[:, pl.ds(n, 128)] = zp
            else:
                zr[:, pl.ds(n, 128)] += zp
        pk[pl.ds(t0 // 2, nt // 2), pl.ds(n0, nn)] = _pack(p.astype(bf16))

    def T(t0, nt):
        xT[:, pl.ds(t0, nt)] = _pack(x_v[pl.ds(t0, nt), :].T)

    def G(t0, nt, n0, nn):
        r = _dot(_unpack(xT[:, pl.ds(t0, nt)]),
                 _unpack(pk[pl.ds(t0 // 2, nt // 2), pl.ds(n0, nn)]))
        for n in range(n0, n0 + nn, 128):
            rp = r[:, n - n0:n - n0 + 128]
            if n not in seen_g:
                seen_g.add(n)
                Gt[:, pl.ds(n, 128)] = rp
            else:
                Gt[:, pl.ds(n, 128)] += rp

    def WQ():
        wqT[...] = _pack(wqkv_v[:, pl.ds(0, D)].T)

    def Q(t0, nt):
        cs = pl.ds(t0, nt)
        q = _dot(_unpack(wqT[...]), _unpack(xT[:, cs]))
        pqT[:, cs] = _pack(_phi(q).astype(bf16))
        for l in range(nt // 128):
            ls = pl.ds(t0 + l * 128, 128)
            zero = _after(q[D - 8:D - 7, l * 128:(l + 1) * 128])
            xb = _unpack(xT[:, ls]).astype(f32)
            m = (jnp.sum(xb, axis=0, keepdims=True) + zero) * (1.0 / D)
            xc = xb - m
            v = jnp.sum(xc * xc, axis=0, keepdims=True) * (1.0 / D)
            hT[:, ls] = _pack((xc * lax.rsqrt(v + 1e-5)).astype(bf16))

    def KV():
        wvT[...] = _pack(wqkv_v[:, pl.ds(2 * D, D)].T)
        r = lax.broadcasted_iota(i32, (128, 128), 0) // DH
        c = lax.broadcasted_iota(i32, (128, 128), 1) // DH
        for g in range(4):
            kvT = _dot(_unpack(wvT[pl.ds(g * 64, 64), :]),
                       Gt[:, pl.ds(g * 128, 128)].astype(bf16))
            kvb[pl.ds(g * 64, 64), :] = _pack(jnp.where(r == c, kvT, 0.0).astype(bf16))

    def MT():
        woT[...] = _pack(wo_v[...].T)
        for g in range(4):
            gs = pl.ds(g * 128, 128)
            mT[:, gs] = _pack(_dot(_unpack(woT[:, gs]),
                                   _unpack(kvb[pl.ds(g * 64, 64), :])).astype(bf16))
        zrow = jnp.sum(zr[...], axis=0, keepdims=True)
        zc[...] = jnp.broadcast_to(zrow, (128, D)).T

    def A(t0, nt):
        js = pl.ds(t0, nt)
        sub = lax.broadcasted_iota(i32, (8, 128), 0)
        m4, m2, m1 = sub < 4, (sub & 2) == 0, (sub & 1) == 0
        tiles = []
        for l in range(nt // 128):
            ls = pl.ds(t0 + l * 128, 128)
            pq = _unpack(pqT[:, ls]).astype(f32)
            pz = pq * zc[...]
            g = jnp.broadcast_to(gT[1:2, ls], (8, 128))
            outs = []
            for hg in range(H // 8):
                h0 = hg * 8
                sv = [pz[(h0 + i) * DH:(h0 + i) * DH + 8]
                      + pz[(h0 + i) * DH + 8:(h0 + i + 1) * DH] for i in range(8)]
                t = [jnp.where(m4, sv[i], sv[i + 4])
                     + pltpu.roll(jnp.where(m4, sv[i + 4], sv[i]), 4, 0) for i in range(4)]
                u = [jnp.where(m2, t[i] + pltpu.roll(t[i], 6, 0),
                               t[i + 2] + pltpu.roll(t[i + 2], 2, 0)) for i in range(2)]
                den = jnp.where(m1, u[0] + pltpu.roll(u[0], 7, 0),
                                u[1] + pltpu.roll(u[1], 1, 0))
                sc = g / (den + 1e-6)
                for i in range(8):
                    b = jnp.broadcast_to(sc[i:i + 1, :], (8, 128))
                    r0 = (h0 + i) * DH
                    outs.append(pq[r0:r0 + 8] * b)
                    outs.append(pq[r0 + 8:r0 + 16] * b)
            tiles.append(jnp.concatenate(outs, axis=0).astype(bf16))
        pqn = jnp.concatenate(tiles, axis=1) if len(tiles) > 1 else tiles[0]
        aT[:, js] = _dot(_unpack(mT[...]), pqn)

    def GWC():
        gwc[...] = jnp.broadcast_to(gw_v[...].astype(f32).reshape(1, D), (128, D)).T

    def U(j, l0=0, nl=0):
        js = pl.ds(j * FC, FC)
        u = _dot(_unpack(hT[...]), w1_v[:, js]) + b12[0:1, js]
        gu[:, js] = _pack(_gelu(u).astype(bf16))
        for i in range(nl):
            ls = pl.ds((l0 + i) * 128, 128)
            r0 = D - 8 * (i + 1)
            zero = _after(u[r0:r0 + 1, (i % 2) * 128:(i % 2 + 1) * 128])
            xb = _unpack(xT[:, ls]).astype(f32)
            gl = jnp.sum(xb * gwc[...], axis=0, keepdims=True) + zero
            gT[1:2, ls] = jax.nn.sigmoid(gl)

    def finish(t0, nt, y):
        js = pl.ds(t0, nt)
        g = gT[1:2, js]
        o = (aT[:, js] + (1.0 - g) * (y + b12[1:2, js])).astype(bf16)
        out_v[js, :] = o.T

    def Y(t0, nt):
        finish(t0, nt, _dot(_unpack(gu[...]), w2_v[:, pl.ds(t0, nt)]))

    def Y128(t0):
        js, km = pl.ds(t0, 128), 1536
        wt = w2_v[pl.ds(km, F - km), js]
        y = _dot(_unpack(gu[:, pl.ds(0, km)]), w2_v[pl.ds(0, km), js])
        ya = _dot(_unpack(gu[pl.ds(0, D // 4), pl.ds(km, F - km)]), wt)
        yb = _dot(_unpack(gu[pl.ds(D // 4, D // 4), pl.ds(km, F - km)]), wt)
        finish(t0, 128, y + jnp.concatenate([ya, yb], axis=0))

    def flush(i, lo, n):
        cp = pltpu.make_async_copy(out_v.at[pl.ds(lo, n)], out_h.at[pl.ds(lo, n)],
                                   out_sems.at[i])
        cp.start()
        return cp

    wait("wk0", "x0")
    K(0, 256, 0, 256); T(0, 256); G(0, 256, 0, 256)

    wait("wk1", "x1")
    K(0, 256, 256, 256); T(256, 256); K(256, 256, 0, 512)
    G(0, 256, 256, 256); G(256, 256, 0, 512)

    wait("gw", "wq", "x2")
    K(512, 512, 0, 512); WQ(); T(512, 512)
    Q(0, 512); Q(512, 512); G(512, 512, 0, 512)

    wait("x3", "x4")
    T(1024, 512); K(1024, 512, 0, 512); Q(1024, 512); G(1024, 512, 0, 512)
    T(1536, 512); K(1536, 512, 0, 512); Q(1536, 512); G(1536, 512, 0, 512)

    wait("wv", "wo", "b1", "b2", "w1")
    b12[0:1, pl.ds(0, F)] = b1_v[...].astype(f32).reshape(1, F)
    U(0); KV(); GWC(); U(1, 0, 4); MT(); U(2, 4, 4); U(3, 8, 4); U(4, 12, 4)
    A(0, 256)

    wait("w2a")
    U(5); U(6)
    b12[1:2, :] = b2_v[...].astype(f32).reshape(1, S)
    Y(0, 256); A(256, 256); Y(256, 256); A(512, 256); Y(512, 256)
    A(768, 256); Y(768, 256); A(1024, 256)

    f0 = flush(0, 0, 1024)
    wait("w2b")
    Y(1024, 256); A(1280, 256); Y(1280, 256); A(1536, 256); Y(1536, 256)
    A(1792, 128); Y128(1792); A(1920, 128)

    f1 = flush(1, 1024, 896)
    f0.wait()
    Y128(1920)
    f2 = flush(2, 1920, 128)
    f1.wait()
    f2.wait()


@jax.jit
def pallas_gated_mix__linear_attn_block__mixer_token_mlp__prompt_kernel(
    A_x: jax.Array,
    A_wqkv: jax.Array,
    A_wo: jax.Array,
    B_x: jax.Array,
    B_w1: jax.Array,
    B_b1: jax.Array,
    B_w2: jax.Array,
    B_b2: jax.Array,
    gate_w: jax.Array,
):
    del B_x
    V = pltpu.VMEM
    scratch = [
        V((S, D), bf16), V((D, 3 * D), bf16), V((D, D), bf16), V((S, F), bf16),
        V((F, S), bf16), V((F,), bf16), V((S,), bf16), V((D,), bf16),
        V((D // 2, D), i32), V((D // 2, D), i32), V((D // 2, D), i32),
        V((D // 2, S), i32), V((D // 2, S), i32), V((D // 2, S), i32), V((S // 2, D), i32),
        V((D, D), f32), V((8, D), f32), V((D, 128), f32), V((D, 128), f32),
        V((8, S), f32), V((8, S), f32), V((D, S), f32),
        V((D // 2, 128), i32), V((D // 2, D), i32), V((D // 2, F), i32), V((S, D), bf16),
        pltpu.SemaphoreType.DMA((16,)), pltpu.SemaphoreType.DMA((3,)),
    ]
    hbm = pl.BlockSpec(memory_space=pl.ANY)
    out = pl.pallas_call(
        _kernel,
        in_specs=[hbm] * 8,
        out_specs=hbm,
        out_shape=jax.ShapeDtypeStruct((S, D), bf16),
        scratch_shapes=scratch,
        compiler_params=pltpu.CompilerParams(
            vmem_limit_bytes=100 * 1024 * 1024,
            disable_semaphore_checks=True,
        ),
    )(A_x.reshape(S, D), A_wqkv, A_wo, B_w1, B_b1, B_w2, B_b2, gate_w)
    return out.reshape(1, S, D)
```

```python
import jax
import jax.numpy as jnp
from jax import lax
import jax.experimental.pallas as pl
import jax.experimental.pallas.tpu as pltpu

S, D, F, H, DH = 2048, 512, 1792, 32, 16
FC = 256
HB, NB = 640, 3
f32, bf16, i32 = jnp.float32, jnp.bfloat16, jnp.int32


def _dot(a, b):
    return lax.dot_general(a, b, (((1,), (0,)), ((), ())), preferred_element_type=f32)


def _phi(t):
    return jnp.where(t > 0, t + 1.0, jnp.exp(t)) + 1e-6


def _gelu(x):
    c = 0.7978845608028654
    return 0.5 * x * (1.0 + jnp.tanh(c * (x + 0.044715 * (x * x * x))))


def _pack(v):
    return pltpu.bitcast(v, i32)


def _unpack(v):
    return pltpu.bitcast(v, bf16)


def _mult128(t):
    return t if isinstance(t, int) else pl.multiple_of(t, 128)


def _after(v):
    return jnp.minimum(jnp.abs(v), 1.0) * 0.0


def _kernel(x_h, wqkv_h, wo_h, w1_h, b1_h, w2_h, b2_h, gw_h,
            out_h,
            x_v, wqkv_v, wo_v, w1_v, w2_v, b1_v, b2_v, gw_v,
            wqT, wvT, woT, xT, hT, pqT, pk,
            Gt, zr, zc, gwc, gT, b12, aT,
            kvb, mT, gu, out_v,
            in_sems, out_sems):

    cps = {}

    def fetch(name, src, dst):
        cps[name] = pltpu.make_async_copy(src, dst, in_sems.at[len(cps)])
        cps[name].start()

    def wait(*names):
        for n in names:
            cps[n].wait()

    def rows(name, h, v, lo, n):
        fetch(name, h.at[pl.ds(lo, n)], v.at[pl.ds(lo, n)])

    def cols(name, h, v, lo, n):
        fetch(name, h.at[:, pl.ds(lo, n)], v.at[:, pl.ds(lo, n)])

    cols("wk0", wqkv_h, wqkv_v, D, 256)
    rows("x0", x_h, x_v, 0, 256)
    cols("wk1", wqkv_h, wqkv_v, D + 256, 256)
    rows("x1", x_h, x_v, 256, 256)
    fetch("gw", gw_h, gw_v)
    cols("wq", wqkv_h, wqkv_v, 0, D)
    rows("x2", x_h, x_v, 512, 512)
    rows("x3", x_h, x_v, 1024, 512)
    rows("x4", x_h, x_v, 1536, 512)
    cols("wv", wqkv_h, wqkv_v, 2 * D, D)
    fetch("wo", wo_h, wo_v)
    fetch("b1", b1_h, b1_v)
    fetch("b2", b2_h, b2_v)
    fetch("w1", w1_h, w1_v)
    fetch("w2", w2_h, w2_v)

    seen_z, seen_g = set(), set()

    def K(t0, nt, n0, nn):
        k = _dot(x_v[pl.ds(t0, nt), :], wqkv_v[:, pl.ds(D + n0, nn)])
        p = _phi(k)
        zpart = jnp.sum(p.reshape(nt // 8, 8, nn), axis=0)
        for n in range(n0, n0 + nn, 128):
            zp = zpart[:, n - n0:n - n0 + 128]
            if n not in seen_z:
                seen_z.add(n)
                zr[:, pl.ds(n, 128)] = zp
            else:
                zr[:, pl.ds(n, 128)] += zp
        pk[pl.ds(t0 // 2, nt // 2), pl.ds(n0, nn)] = _pack(p.astype(bf16))

    def T(t0, nt):
        xT[:, pl.ds(t0, nt)] = _pack(x_v[pl.ds(t0, nt), :].T)

    def G(t0, nt, n0, nn):
        r = _dot(_unpack(xT[:, pl.ds(t0, nt)]),
                 _unpack(pk[pl.ds(t0 // 2, nt // 2), pl.ds(n0, nn)]))
        for n in range(n0, n0 + nn, 128):
            rp = r[:, n - n0:n - n0 + 128]
            if n not in seen_g:
                seen_g.add(n)
                Gt[:, pl.ds(n, 128)] = rp
            else:
                Gt[:, pl.ds(n, 128)] += rp

    def WQ():
        wqT[...] = _pack(wqkv_v[:, pl.ds(0, D)].T)

    def Q(t0, nt):
        cs = pl.ds(t0, nt)
        q = _dot(_unpack(wqT[...]), _unpack(xT[:, cs]))
        pqT[:, cs] = _pack(_phi(q).astype(bf16))
        for l in range(nt // 128):
            ls = pl.ds(t0 + l * 128, 128)
            zero = _after(q[D - 8:D - 7, l * 128:(l + 1) * 128])
            xb = _unpack(xT[:, ls]).astype(f32)
            m = (jnp.sum(xb, axis=0, keepdims=True) + zero) * (1.0 / D)
            xc = xb - m
            v = jnp.sum(xc * xc, axis=0, keepdims=True) * (1.0 / D)
            hT[:, ls] = _pack((xc * lax.rsqrt(v + 1e-5)).astype(bf16))

    def KV():
        wvT[...] = _pack(wqkv_v[:, pl.ds(2 * D, D)].T)
        r = lax.broadcasted_iota(i32, (128, 128), 0) // DH
        c = lax.broadcasted_iota(i32, (128, 128), 1) // DH
        for g in range(4):
            kvT = _dot(_unpack(wvT[pl.ds(g * 64, 64), :]),
                       Gt[:, pl.ds(g * 128, 128)].astype(bf16))
            kvb[pl.ds(g * 64, 64), :] = _pack(jnp.where(r == c, kvT, 0.0).astype(bf16))

    def MT():
        woT[...] = _pack(wo_v[...].T)
        for g in range(4):
            gs = pl.ds(g * 128, 128)
            mT[:, gs] = _pack(_dot(_unpack(woT[:, gs]),
                                   _unpack(kvb[pl.ds(g * 64, 64), :])).astype(bf16))
        zrow = jnp.sum(zr[...], axis=0, keepdims=True)
        zc[...] = jnp.broadcast_to(zrow, (128, D)).T

    def A(t0, nt):
        js = pl.ds(t0, nt)
        sub = lax.broadcasted_iota(i32, (8, 128), 0)
        m4, m2, m1 = sub < 4, (sub & 2) == 0, (sub & 1) == 0
        tiles = []
        for l in range(nt // 128):
            ls = pl.ds(_mult128(t0 + l * 128), 128)
            pq = _unpack(pqT[:, ls]).astype(f32)
            pz = pq * zc[...]
            g = jnp.broadcast_to(gT[1:2, ls], (8, 128))
            outs = []
            for hg in range(H // 8):
                h0 = hg * 8
                sv = [pz[(h0 + i) * DH:(h0 + i) * DH + 8]
                      + pz[(h0 + i) * DH + 8:(h0 + i + 1) * DH] for i in range(8)]
                t = [jnp.where(m4, sv[i], sv[i + 4])
                     + pltpu.roll(jnp.where(m4, sv[i + 4], sv[i]), 4, 0) for i in range(4)]
                u = [jnp.where(m2, t[i] + pltpu.roll(t[i], 6, 0),
                               t[i + 2] + pltpu.roll(t[i + 2], 2, 0)) for i in range(2)]
                den = jnp.where(m1, u[0] + pltpu.roll(u[0], 7, 0),
                                u[1] + pltpu.roll(u[1], 1, 0))
                sc = g / (den + 1e-6)
                for i in range(8):
                    b = jnp.broadcast_to(sc[i:i + 1, :], (8, 128))
                    r0 = (h0 + i) * DH
                    outs.append(pq[r0:r0 + 8] * b)
                    outs.append(pq[r0 + 8:r0 + 16] * b)
            tiles.append(jnp.concatenate(outs, axis=0).astype(bf16))
        pqn = jnp.concatenate(tiles, axis=1) if len(tiles) > 1 else tiles[0]
        aT[:, js] = _dot(_unpack(mT[...]), pqn)

    def GWC():
        gwc[...] = jnp.broadcast_to(gw_v[...].astype(f32).reshape(1, D), (128, D)).T

    def U(j, l0=0, nl=0):
        js = pl.ds(j * FC, FC)
        u = _dot(_unpack(hT[...]), w1_v[:, js]) + b12[0:1, js]
        gu[:, js] = _pack(_gelu(u).astype(bf16))
        for i in range(nl):
            ls = pl.ds((l0 + i) * 128, 128)
            r0 = D - 8 * (i + 1)
            zero = _after(u[r0:r0 + 1, (i % 2) * 128:(i % 2 + 1) * 128])
            xb = _unpack(xT[:, ls]).astype(f32)
            gl = jnp.sum(xb * gwc[...], axis=0, keepdims=True) + zero
            gT[1:2, ls] = jax.nn.sigmoid(gl)

    def finish(t0, nt, y):
        js = pl.ds(t0, nt)
        g = gT[1:2, js]
        o = (aT[:, js] + (1.0 - g) * (y + b12[1:2, js])).astype(bf16)
        out_v[js, :] = o.T

    def Y(t0, nt):
        finish(t0, nt, _dot(_unpack(gu[...]), w2_v[:, pl.ds(t0, nt)]))

    def Y128(t0):
        js, km = pl.ds(t0, 128), 1536
        wt = w2_v[pl.ds(km, F - km), js]
        y = _dot(_unpack(gu[:, pl.ds(0, km)]), w2_v[pl.ds(0, km), js])
        ya = _dot(_unpack(gu[pl.ds(0, D // 4), pl.ds(km, F - km)]), wt)
        yb = _dot(_unpack(gu[pl.ds(D // 4, D // 4), pl.ds(km, F - km)]), wt)
        finish(t0, 128, y + jnp.concatenate([ya, yb], axis=0))

    def flush(i, lo, n):
        return pltpu.make_async_copy(out_v.at[pl.ds(lo, n)], out_h.at[pl.ds(lo, n)],
                                     out_sems.at[i])

    wait("wk0", "x0")
    K(0, 256, 0, 256); T(0, 256); G(0, 256, 0, 256)

    wait("wk1", "x1")
    K(0, 256, 256, 256); T(256, 256); K(256, 256, 0, 512)
    G(0, 256, 256, 256); G(256, 256, 0, 512)

    wait("gw", "wq", "x2")
    K(512, 512, 0, 512); WQ(); T(512, 512)
    Q(0, 512); Q(512, 512); G(512, 512, 0, 512)

    wait("x3", "x4")
    T(1024, 512); K(1024, 512, 0, 512); Q(1024, 512); G(1024, 512, 0, 512)
    T(1536, 512); K(1536, 512, 0, 512); Q(1536, 512); G(1536, 512, 0, 512)

    wait("wv", "wo", "b1", "b2", "w1")
    b12[0:1, pl.ds(0, F)] = b1_v[...].astype(f32).reshape(1, F)
    U(0); KV(); GWC(); U(1, 0, 4); MT(); U(2, 4, 4); U(3, 8, 4); U(4, 12, 4)
    U(5); U(6)
    b12[1:2, :] = b2_v[...].astype(f32).reshape(1, S)
    A(0, 128)

    wait("w2")
    def body(i, carry):
        b0 = pl.multiple_of(i * HB, 128)
        o = lambda k: pl.multiple_of(b0 + k, 128)
        Y128(o(0)); A(o(128), 256); Y(o(128), 256); A(o(384), 256); Y(o(384), 256)
        A(o(640), 128)
        flush(i, b0, HB).start()
        return carry

    lax.fori_loop(0, NB, body, 0)
    Y128(NB * HB)
    flush(NB, NB * HB, S - NB * HB).start()
    for i in range(NB):
        flush(i, i * HB, HB).wait()
    flush(NB, NB * HB, S - NB * HB).wait()


@jax.jit
def pallas_gated_mix__linear_attn_block__mixer_token_mlp__prompt_kernel(
    A_x: jax.Array,
    A_wqkv: jax.Array,
    A_wo: jax.Array,
    B_x: jax.Array,
    B_w1: jax.Array,
    B_b1: jax.Array,
    B_w2: jax.Array,
    B_b2: jax.Array,
    gate_w: jax.Array,
):
    del B_x
    V = pltpu.VMEM
    scratch = [
        V((S, D), bf16), V((D, 3 * D), bf16), V((D, D), bf16), V((S, F), bf16),
        V((F, S), bf16), V((F,), bf16), V((S,), bf16), V((D,), bf16),
        V((D // 2, D), i32), V((D // 2, D), i32), V((D // 2, D), i32),
        V((D // 2, S), i32), V((D // 2, S), i32), V((D // 2, S), i32), V((S // 2, D), i32),
        V((D, D), f32), V((8, D), f32), V((D, 128), f32), V((D, 128), f32),
        V((8, S), f32), V((8, S), f32), V((D, S), f32),
        V((D // 2, 128), i32), V((D // 2, D), i32), V((D // 2, F), i32), V((S, D), bf16),
        pltpu.SemaphoreType.DMA((15,)), pltpu.SemaphoreType.DMA((4,)),
    ]
    hbm = pl.BlockSpec(memory_space=pl.ANY)
    out = pl.pallas_call(
        _kernel,
        in_specs=[hbm] * 8,
        out_specs=hbm,
        out_shape=jax.ShapeDtypeStruct((S, D), bf16),
        scratch_shapes=scratch,
        compiler_params=pltpu.CompilerParams(
            vmem_limit_bytes=100 * 1024 * 1024,
            disable_semaphore_checks=True,
        ),
    )(A_x.reshape(S, D), A_wqkv, A_wo, B_w1, B_b1, B_w2, B_b2, gate_w)
    return out.reshape(1, S, D)
```

```python
import jax
import jax.numpy as jnp
from jax import lax
import jax.experimental.pallas as pl
import jax.experimental.pallas.tpu as pltpu

S, D, F, H, DH = 2048, 512, 1792, 32, 16
FC = 256
HB, NB = 640, 3
f32, bf16, i32 = jnp.float32, jnp.bfloat16, jnp.int32


def _dot(a, b):
    return lax.dot_general(a, b, (((1,), (0,)), ((), ())), preferred_element_type=f32)


def _phi(t):
    return jnp.where(t > 0, t + 1.0, jnp.exp(t)) + 1e-6


def _gelu(x):
    c = 0.7978845608028654
    return 0.5 * x * (1.0 + jnp.tanh(c * (x + 0.044715 * (x * x * x))))


def _pack(v):
    return pltpu.bitcast(v, i32)


def _unpack(v):
    return pltpu.bitcast(v, bf16)


def _mult128(t):
    return t if isinstance(t, int) else pl.multiple_of(t, 128)


def _after(v):
    return jnp.minimum(jnp.abs(v), 1.0) * 0.0


def _kernel(x_h, wqkv_h, wo_h, w1_h, b1_h, w2_h, b2_h, gw_h,
            out_h,
            x_v, wqkv_v, wo_v, w1_v, w2_v, b1_v, b2_v, gw_v,
            wqT, wvT, woT, xT, hT, pqT, pk,
            Gt, zr, zc, gwc, gT, b12, aT,
            kvb, mT, gu, out_v,
            in_sems, out_sems):

    cps = {}

    def fetch(name, src, dst):
        cps[name] = pltpu.make_async_copy(src, dst, in_sems.at[len(cps)])
        cps[name].start()

    def wait(*names):
        for n in names:
            cps[n].wait()

    def rows(name, h, v, lo, n):
        fetch(name, h.at[pl.ds(lo, n)], v.at[pl.ds(lo, n)])

    def cols(name, h, v, lo, n):
        fetch(name, h.at[:, pl.ds(lo, n)], v.at[:, pl.ds(lo, n)])

    cols("wk0", wqkv_h, wqkv_v, D, 256)
    rows("x0", x_h, x_v, 0, 256)
    cols("wk1", wqkv_h, wqkv_v, D + 256, 256)
    rows("x1", x_h, x_v, 256, 384)
    fetch("gw", gw_h, gw_v)
    cols("wq", wqkv_h, wqkv_v, 0, D)
    rows("x2", x_h, x_v, 640, S - 640)
    cols("wv", wqkv_h, wqkv_v, 2 * D, D)
    fetch("wo", wo_h, wo_v)
    fetch("b1", b1_h, b1_v)
    fetch("b2", b2_h, b2_v)
    fetch("w1", w1_h, w1_v)
    fetch("w2", w2_h, w2_v)

    seen_z, seen_g = set(), set()

    def K(t0, nt, n0, nn):
        k = _dot(x_v[pl.ds(t0, nt), :], wqkv_v[:, pl.ds(D + n0, nn)])
        p = _phi(k)
        zpart = jnp.sum(p.reshape(nt // 8, 8, nn), axis=0)
        for n in range(n0, n0 + nn, 128):
            zp = zpart[:, n - n0:n - n0 + 128]
            if n not in seen_z:
                seen_z.add(n)
                zr[:, pl.ds(n, 128)] = zp
            else:
                zr[:, pl.ds(n, 128)] += zp
        pk[pl.ds(t0 // 2, nt // 2), pl.ds(n0, nn)] = _pack(p.astype(bf16))

    def T(t0, nt):
        xT[:, pl.ds(t0, nt)] = _pack(x_v[pl.ds(t0, nt), :].T)

    def G(t0, nt, n0, nn):
        r = _dot(_unpack(xT[:, pl.ds(t0, nt)]),
                 _unpack(pk[pl.ds(t0 // 2, nt // 2), pl.ds(n0, nn)]))
        for n in range(n0, n0 + nn, 128):
            rp = r[:, n - n0:n - n0 + 128]
            if n not in seen_g:
                seen_g.add(n)
                Gt[:, pl.ds(n, 128)] = rp
            else:
                Gt[:, pl.ds(n, 128)] += rp

    def WQ():
        wqT[...] = _pack(wqkv_v[:, pl.ds(0, D)].T)

    def Q(t0, nt):
        cs = pl.ds(t0, nt)
        q = _dot(_unpack(wqT[...]), _unpack(xT[:, cs]))
        pqT[:, cs] = _pack(_phi(q).astype(bf16))
        for l in range(nt // 128):
            ls = pl.ds(t0 + l * 128, 128)
            zero = _after(q[D - 8:D - 7, l * 128:(l + 1) * 128])
            xb = _unpack(xT[:, ls]).astype(f32)
            m = (jnp.sum(xb, axis=0, keepdims=True) + zero) * (1.0 / D)
            xc = xb - m
            v = jnp.sum(xc * xc, axis=0, keepdims=True) * (1.0 / D)
            hT[:, ls] = _pack((xc * lax.rsqrt(v + 1e-5)).astype(bf16))

    def KV():
        wvT[...] = _pack(wqkv_v[:, pl.ds(2 * D, D)].T)
        r = lax.broadcasted_iota(i32, (128, 128), 0) // DH
        c = lax.broadcasted_iota(i32, (128, 128), 1) // DH
        for g in range(4):
            kvT = _dot(_unpack(wvT[pl.ds(g * 64, 64), :]),
                       Gt[:, pl.ds(g * 128, 128)].astype(bf16))
            kvb[pl.ds(g * 64, 64), :] = _pack(jnp.where(r == c, kvT, 0.0).astype(bf16))

    def MT():
        woT[...] = _pack(wo_v[...].T)
        for g in range(4):
            gs = pl.ds(g * 128, 128)
            mT[:, gs] = _pack(_dot(_unpack(woT[:, gs]),
                                   _unpack(kvb[pl.ds(g * 64, 64), :])).astype(bf16))
        zrow = jnp.sum(zr[...], axis=0, keepdims=True)
        zc[...] = jnp.broadcast_to(zrow, (128, D)).T

    def A(t0, nt):
        js = pl.ds(t0, nt)
        sub = lax.broadcasted_iota(i32, (8, 128), 0)
        m4, m2, m1 = sub < 4, (sub & 2) == 0, (sub & 1) == 0
        tiles = []
        for l in range(nt // 128):
            ls = pl.ds(_mult128(t0 + l * 128), 128)
            pq = _unpack(pqT[:, ls]).astype(f32)
            pz = pq * zc[...]
            g = jnp.broadcast_to(gT[1:2, ls], (8, 128))
            outs = []
            for hg in range(H // 8):
                h0 = hg * 8
                sv = [pz[(h0 + i) * DH:(h0 + i) * DH + 8]
                      + pz[(h0 + i) * DH + 8:(h0 + i + 1) * DH] for i in range(8)]
                t = [jnp.where(m4, sv[i], sv[i + 4])
                     + pltpu.roll(jnp.where(m4, sv[i + 4], sv[i]), 4, 0) for i in range(4)]
                u = [jnp.where(m2, t[i] + pltpu.roll(t[i], 6, 0),
                               t[i + 2] + pltpu.roll(t[i + 2], 2, 0)) for i in range(2)]
                den = jnp.where(m1, u[0] + pltpu.roll(u[0], 7, 0),
                                u[1] + pltpu.roll(u[1], 1, 0))
                sc = g / (den + 1e-6)
                for i in range(8):
                    b = jnp.broadcast_to(sc[i:i + 1, :], (8, 128))
                    r0 = (h0 + i) * DH
                    outs.append(pq[r0:r0 + 8] * b)
                    outs.append(pq[r0 + 8:r0 + 16] * b)
            tiles.append(jnp.concatenate(outs, axis=0).astype(bf16))
        pqn = jnp.concatenate(tiles, axis=1) if len(tiles) > 1 else tiles[0]
        aT[:, js] = _dot(_unpack(mT[...]), pqn)

    def GWC():
        gwc[...] = jnp.broadcast_to(gw_v[...].astype(f32).reshape(1, D), (128, D)).T

    def U(j, l0=0, nl=0):
        js = pl.ds(j * FC, FC)
        u = _dot(_unpack(hT[...]), w1_v[:, js]) + b12[0:1, js]
        gu[:, js] = _pack(_gelu(u).astype(bf16))
        for i in range(nl):
            ls = pl.ds((l0 + i) * 128, 128)
            r0 = D - 8 * (i + 1)
            zero = _after(u[r0:r0 + 1, (i % 2) * 128:(i % 2 + 1) * 128])
            xb = _unpack(xT[:, ls]).astype(f32)
            gl = jnp.sum(xb * gwc[...], axis=0, keepdims=True) + zero
            gT[1:2, ls] = jax.nn.sigmoid(gl)

    def finish(t0, nt, y):
        js = pl.ds(t0, nt)
        g = gT[1:2, js]
        o = (aT[:, js] + (1.0 - g) * (y + b12[1:2, js])).astype(bf16)
        out_v[js, :] = o.T

    def Y(t0, nt):
        finish(t0, nt, _dot(_unpack(gu[...]), w2_v[:, pl.ds(t0, nt)]))

    def Y128(t0):
        js, km = pl.ds(t0, 128), 1536
        wt = w2_v[pl.ds(km, F - km), js]
        y = _dot(_unpack(gu[:, pl.ds(0, km)]), w2_v[pl.ds(0, km), js])
        ya = _dot(_unpack(gu[pl.ds(0, D // 4), pl.ds(km, F - km)]), wt)
        yb = _dot(_unpack(gu[pl.ds(D // 4, D // 4), pl.ds(km, F - km)]), wt)
        finish(t0, 128, y + jnp.concatenate([ya, yb], axis=0))

    def flush(i, lo, n):
        return pltpu.make_async_copy(out_v.at[pl.ds(lo, n)], out_h.at[pl.ds(lo, n)],
                                     out_sems.at[i])

    wait("wk0", "x0")
    K(0, 256, 0, 256); T(0, 256); G(0, 256, 0, 256)

    wait("wk1", "x1")
    K(0, 256, 256, 256); T(256, 384); K(256, 384, 0, 512)
    G(0, 256, 256, 256); G(256, 384, 0, 512)

    wait("gw", "wq", "x2")
    K(640, 384, 0, 512); WQ(); T(640, 384)
    Q(0, 512); Q(512, 512); G(640, 384, 0, 512)
    T(1024, 512); K(1024, 512, 0, 512); Q(1024, 512); G(1024, 512, 0, 512)
    T(1536, 512); K(1536, 512, 0, 512); Q(1536, 512); G(1536, 512, 0, 512)

    wait("wv", "wo", "b1", "b2", "w1")
    b12[0:1, pl.ds(0, F)] = b1_v[...].astype(f32).reshape(1, F)
    U(0); KV(); GWC(); U(1, 0, 4); MT(); U(2, 4, 4); U(3, 8, 4); U(4, 12, 4)
    U(5); U(6)
    b12[1:2, :] = b2_v[...].astype(f32).reshape(1, S)
    A(0, 128)

    wait("w2")
    def body(i, carry):
        b0 = pl.multiple_of(i * HB, 128)
        o = lambda k: pl.multiple_of(b0 + k, 128)
        Y128(o(0)); A(o(128), 256); Y(o(128), 256); A(o(384), 256); Y(o(384), 256)
        A(o(640), 128)
        flush(i, b0, HB).start()
        return carry

    lax.fori_loop(0, NB, body, 0)
    Y128(NB * HB)
    flush(NB, NB * HB, S - NB * HB).start()
    for i in range(NB):
        flush(i, i * HB, HB).wait()
    flush(NB, NB * HB, S - NB * HB).wait()


@jax.jit
def pallas_gated_mix__linear_attn_block__mixer_token_mlp__prompt_kernel(
    A_x: jax.Array,
    A_wqkv: jax.Array,
    A_wo: jax.Array,
    B_x: jax.Array,
    B_w1: jax.Array,
    B_b1: jax.Array,
    B_w2: jax.Array,
    B_b2: jax.Array,
    gate_w: jax.Array,
):
    del B_x
    V = pltpu.VMEM
    scratch = [
        V((S, D), bf16), V((D, 3 * D), bf16), V((D, D), bf16), V((S, F), bf16),
        V((F, S), bf16), V((F,), bf16), V((S,), bf16), V((D,), bf16),
        V((D // 2, D), i32), V((D // 2, D), i32), V((D // 2, D), i32),
        V((D // 2, S), i32), V((D // 2, S), i32), V((D // 2, S), i32), V((S // 2, D), i32),
        V((D, D), f32), V((8, D), f32), V((D, 128), f32), V((D, 128), f32),
        V((8, S), f32), V((8, S), f32), V((D, S), f32),
        V((D // 2, 128), i32), V((D // 2, D), i32), V((D // 2, F), i32), V((S, D), bf16),
        pltpu.SemaphoreType.DMA((13,)), pltpu.SemaphoreType.DMA((4,)),
    ]
    hbm = pl.BlockSpec(memory_space=pl.ANY)
    out = pl.pallas_call(
        _kernel,
        in_specs=[hbm] * 8,
        out_specs=hbm,
        out_shape=jax.ShapeDtypeStruct((S, D), bf16),
        scratch_shapes=scratch,
        compiler_params=pltpu.CompilerParams(
            vmem_limit_bytes=100 * 1024 * 1024,
            disable_semaphore_checks=True,
        ),
    )(A_x.reshape(S, D), A_wqkv, A_wo, B_w1, B_b1, B_w2, B_b2, gate_w)
    return out.reshape(1, S, D)
```
